```python
import os as _os
_os.environ.setdefault("JAX_PLATFORMS", "cpu")
import jax
import jax.numpy as jnp

def _softmax(x, axis=-1):
    return jax.nn.softmax(x, axis=axis)
def _gelu(x):
    return jax.nn.gelu(x, approximate=True)
def _silu(x):
    return jax.nn.silu(x)
def _sigmoid(x):
    return jax.nn.sigmoid(x)
def _layernorm(x, axis=-1, eps=1e-5):
    m = jnp.mean(x, axis=axis, keepdims=True)
    v = jnp.var(x, axis=axis, keepdims=True)
    return (x - m) / jnp.sqrt(v + eps)
def _scatter_add(tgt, idx, src, axis=0):
    return tgt.at[idx].add(src)
def _segment_sum(src, seg, n):
    return jax.ops.segment_sum(src, seg, n)
class _Rng:
    def __init__(self, key):
        self._k = key
    def _next(self):
        self._k, sub = jax.random.split(self._k)
        return sub
    def normal(self, shape):
        return jax.random.normal(self._next(), shape, dtype=jnp.bfloat16)
    def randint(self, lo, hi, shape):
        return jax.random.randint(self._next(), shape, lo, hi, dtype=jnp.int32)
    def uniform(self, shape, lo=0.0, hi=1.0):
        return jax.random.uniform(self._next(), shape, jnp.bfloat16, lo, hi)
    def permutation(self, n):
        return jax.random.permutation(self._next(), n)


kernel_name = 'parallel_sum__linear_kernel_hedgehog__dense_activation_gelu__prompt'

def setup_inputs():
    _rng = _Rng(jax.random.key(int.from_bytes(__import__("os").urandom(4), "little")))
    _w = (lambda a: (lambda t: t.astype(jnp.bfloat16) if jnp.issubdtype(t.dtype, jnp.floating) else t)(jnp.asarray(a)))
    def _A_setup():
        B, S, D, H = 1, 2048, 448, 16
        Dh = D // H
        return {
            "x": _w((lambda *s: _rng.normal(s) * 0.05)(B, S, D)),
            "wqkv": _w((lambda *s: _rng.normal(s) * 0.2)(D, 3 * D)),
            "w_phi": _w((lambda *s: _rng.normal(s) * 0.2)(H, Dh, Dh) * (Dh ** -0.5)),
            "wo": _w((lambda *s: _rng.normal(s) * 0.05)(D, D)),
        }
    _A_in = _A_setup()

    def _B_setup():
        B, S, D, F = 1, 2048, 448, 1792
        return {
            "x": _w((lambda *s: _rng.normal(s) * 0.05)(B, S, D)),
            "w1": _w((lambda *s: _rng.normal(s) * 0.2)(D, F) * (D ** -0.5)),
            "b1": _w((lambda *s: _rng.normal(s) * 0.2)(F) * 0.01),
            "w2": _w((lambda *s: _rng.normal(s) * 0.2)(F, D) * (F ** -0.5)),
            "b2": _w((lambda *s: _rng.normal(s) * 0.05)(D) * 0.01),
        }
    _B_in = _B_setup()

    return {
        "A_x": _A_in["x"],
        "A_wqkv": _A_in["wqkv"],
        "A_w_phi": _A_in["w_phi"],
        "A_wo": _A_in["wo"],
        "B_x": _B_in["x"],
        "B_w1": _B_in["w1"],
        "B_b1": _B_in["b1"],
        "B_w2": _B_in["w2"],
        "B_b2": _B_in["b2"],
    }

def reference(A_x, A_wqkv, A_w_phi, A_wo, B_x, B_w1, B_b1, B_w2, B_b2):
    def _A_ref(x, wqkv, w_phi, wo):
        B, S, D = x.shape
        H = 16; Dh = D // H
        qkv = (lambda x, *d: x.transpose(*d))((x @ wqkv).reshape(B, S, 3, H, Dh), 2, 0, 3, 1, 4)
        q, k, v = qkv[0], qkv[1], qkv[2]
        pq = jnp.einsum("bhsd,hdf->bhsf", q, w_phi)
        pk = jnp.einsum("bhsd,hdf->bhsf", k, w_phi)
        phi_q = jnp.concatenate([_softmax(pq, axis=-1), _softmax(-pq, axis=-1)], axis=-1)
        phi_k = jnp.concatenate([_softmax(pk, axis=-1), _softmax(-pk, axis=-1)], axis=-1)
        kv = jnp.einsum("bhsf,bhsd->bhfd", phi_k, v)
        z  = jnp.einsum("bhsf->bhf", phi_k)
        num = jnp.einsum("bhqf,bhfd->bhqd", phi_q, kv)
        den = jnp.einsum("bhqf,bhf->bhq", phi_q, z)[..., None] + 1e-6
        o = num / den
        return (lambda x, *d: x.transpose(*d))(o, 0, 2, 1, 3).reshape(B, S, D) @ wo

    def _B_ref(x, w1, b1, w2, b2):
        h = jnp.einsum("bsd,df->bsf", x, w1) + b1
        h = _gelu(h)
        return jnp.einsum("bsf,fd->bsd", h, w2) + b2

    x = A_x
    xn = _layernorm(x, axis=-1)
    return x + _A_ref(xn, A_wqkv, A_w_phi, A_wo) + _B_ref(xn, B_w1, B_b1, B_w2, B_b2)
```

```python
import jax
import jax.numpy as jnp
from jax import lax
import jax.experimental.pallas as pl
import jax.experimental.pallas.tpu as pltpu

S, D, H, DH, F = 2048, 448, 16, 28, 1792
HP = 32
DP = H * HP
T = 256
NTILE = S // T
LOG2E = 1.4426950408889634
f32 = jnp.float32
bf16 = jnp.bfloat16


def _nt(a, b):
    return lax.dot_general(a, b, (((1,), (1,)), ((), ())), preferred_element_type=f32)


def _tn(a, b):
    return lax.dot_general(a, b, (((0,), (0,)), ((), ())), preferred_element_type=f32)


def _nn(a, b):
    return jnp.dot(a, b, preferred_element_type=f32)


def _kernel(x_hbm, wqkv_hbm, wphi_hbm, wo_hbm, w1_hbm, b1_hbm, w2T_hbm, b2_hbm, out_hbm,
            x_v, wqkv_v, wphi_v, wo_v, w1_v, b1_v, w2T, b2_v, out_v, xn_v,
            wqT, wkT, wvT, woT, a_pad, kv_acc, kvp, kvn,
            sem_x, sem_w, sem_o):
    def x_copy(i):
        return pltpu.make_async_copy(x_hbm.at[:, pl.ds(i * T, T)], x_v.at[:, pl.ds(i * T, T)], sem_x.at[i])

    def o_copy(i):
        return pltpu.make_async_copy(out_v.at[:, pl.ds(i * T, T)], out_hbm.at[:, pl.ds(i * T, T)], sem_o.at[i])

    c_wqkv = pltpu.make_async_copy(wqkv_hbm, wqkv_v, sem_w.at[0])
    c_w2 = pltpu.make_async_copy(w2T_hbm, w2T, sem_w.at[1])
    c_wo = pltpu.make_async_copy(wo_hbm, wo_v, sem_w.at[2])
    c_w1 = pltpu.make_async_copy(w1_hbm, w1_v, sem_w.at[3])
    c_wphi = pltpu.make_async_copy(wphi_hbm, wphi_v, sem_w.at[4])
    c_b1 = pltpu.make_async_copy(b1_hbm, b1_v, sem_w.at[5])
    c_b2 = pltpu.make_async_copy(b2_hbm, b2_v, sem_w.at[6])

    c_wphi.start()
    c_wqkv.start()
    x_copy(0).start()
    c_b1.start()
    c_b2.start()

    a_pad[...] = jnp.zeros_like(a_pad)
    rr = lax.broadcasted_iota(jnp.int32, (DP, DP), 0)
    cc = lax.broadcasted_iota(jnp.int32, (DP, DP), 1)
    lo = (rr >> 5) * DH
    f_in = rr & 31
    bd_v = jnp.where((cc == lo + f_in) & (f_in < DH), 1.0, 0.0).astype(bf16)
    r32 = lax.broadcasted_iota(jnp.int32, (HP, 128), 0)
    c32 = lax.broadcasted_iota(jnp.int32, (HP, 128), 1)
    i_ext = jnp.where(c32 == jnp.where(r32 < DH, r32, r32 - 4), 1.0, 0.0).astype(bf16)
    c_wphi.wait()
    for d in range(DH):
        a_pad[pl.ds(64 + d, H, stride=DH), 0:DH] = wphi_v[d].astype(f32)
    t32_q = _nt(i_ext, a_pad[64:576, :].astype(bf16))
    t32_k = _nt(i_ext, a_pad[0:512, :].astype(bf16))

    def bd(t32, off):
        tiled = jnp.broadcast_to(t32[None], (H, HP, DP)).reshape(DP, DP)
        m = (cc >= lo + off) & (cc < lo + off + DH)
        return jnp.where(m, tiled, 0.0).astype(bf16)

    bd_q = bd(t32_q, 0)
    bd_k = bd(t32_k, 64)

    for i in range(1, NTILE):
        x_copy(i).start()
    c_wqkv.wait()
    c_wo.start()
    c_w1.start()
    c_w2.start()

    def fold(bdm, base, off, dst, scale):
        for g in range(4):
            lo_c = off + 112 * g
            t0, t1 = lo_c // 128, (lo_c + 111) // 128
            c0 = t0 * 128
            c1 = min((t1 + 1) * 128, 3 * D - base)
            w = _nt(bdm[128 * g:128 * (g + 1), c0:c1], wqkv_v[:, base + c0:base + c1])
            if scale is not None:
                w = w * scale
            dst[128 * g:128 * (g + 1), :] = w.astype(bf16)

    fold(bd_k, 384, 64, wkT, LOG2E)
    fold(bd_v, 896, 0, wvT, None)
    fold(bd_q, 0, 0, wqT, LOG2E)

    kv_acc[...] = jnp.zeros_like(kv_acc)

    sub = lax.broadcasted_iota(jnp.int32, (H, HP, T), 1)

    def phase1(i, carry):
        r = pl.multiple_of(i * T, T)
        pltpu.make_async_copy(x_hbm.at[:, pl.ds(r, T)], x_v.at[:, pl.ds(r, T)], sem_x.at[i]).wait()
        x = x_v[:, pl.ds(r, T)].astype(f32)
        m = jnp.mean(x, axis=0, keepdims=True)
        xc = x - m
        var = jnp.mean(xc * xc, axis=0, keepdims=True)
        xn = (xc * lax.rsqrt(var + 1e-5)).astype(bf16)
        xn_v[:, pl.ds(r, T)] = xn
        p3 = _nn(wkT[...], xn).reshape(H, HP, T)
        v3 = _nn(wvT[...], xn).reshape(H, HP, T)
        mx = jnp.max(p3, axis=1, keepdims=True)
        mn = jnp.min(p3, axis=1, keepdims=True)
        ep = jnp.exp2(p3 - mx)
        en = jnp.exp2(mn - p3)
        real = sub < DH
        sp = jnp.sum(jnp.where(real, ep, 0.0), axis=1, keepdims=True)
        sn = jnp.sum(jnp.where(real, en, 0.0), axis=1, keepdims=True)
        php = (ep * (1.0 / sp)).astype(bf16).reshape(DP, T)
        phn = (en * (1.0 / sn)).astype(bf16).reshape(DP, T)
        vT = jnp.where(sub == DH, 1.0, v3).astype(bf16).reshape(DP, T)
        for g in range(4):
            sl = slice(128 * g, 128 * (g + 1))
            kv_acc[g, :, 0:128] += _nt(vT[sl], php[sl])
            kv_acc[g, :, 128:256] += _nt(vT[sl], phn[sl])
        return carry

    lax.fori_loop(0, NTILE, phase1, 0)

    rd = lax.broadcasted_iota(jnp.int32, (128, 128), 0)
    cf = lax.broadcasted_iota(jnp.int32, (128, 128), 1)
    own = ((rd >> 5) == (cf >> 5)) & ((cf & 31) < DH)
    ones_row = (rd & 31) == DH + 1
    for g in range(4):
        kvp[g] = jnp.where(own, jnp.where(ones_row, 1.0, kv_acc[g, :, 0:128]), 0.0).astype(bf16)
        kvn[g] = jnp.where(own, jnp.where(ones_row, 1.0, kv_acc[g, :, 128:256]), 0.0).astype(bf16)

    c_wo.wait()
    c_b2.wait()
    wo_pad = _nn(bd_v[:, 0:448], wo_v[...])
    rw = lax.broadcasted_iota(jnp.int32, (DP, D), 0)
    wo_pad = jnp.where(rw == 30, b2_v[...].astype(f32).reshape(1, D), wo_pad)
    woT[0:384, :] = wo_pad[:, 0:384].T.astype(bf16)
    tail = jnp.concatenate([wo_pad[:, 384:448], jnp.zeros((512, 64), f32)], axis=1)
    woT[384:448, :] = tail.T[0:64].astype(bf16)
    c_w1.wait()
    c_w2.wait()
    c_b1.wait()
    b1 = b1_v[...].astype(f32).reshape(1, F)
    row = lax.broadcasted_iota(jnp.int32, (DP, T), 0)

    def phase2(i, carry):
        r = pl.multiple_of(i * T, T)
        xn = xn_v[:, pl.ds(r, T)]
        p3 = _nn(wqT[...], xn).reshape(H, HP, T)
        mx = jnp.max(p3, axis=1, keepdims=True)
        mn = jnp.min(p3, axis=1, keepdims=True)
        ep = jnp.exp2(p3 - mx).astype(bf16).reshape(DP, T)
        en = jnp.exp2(mn - p3).astype(bf16).reshape(DP, T)
        nump = jnp.concatenate([_nn(kvp[g], ep[128 * g:128 * (g + 1)]) for g in range(4)], axis=0).reshape(H, HP, T)
        numn = jnp.concatenate([_nn(kvn[g], en[128 * g:128 * (g + 1)]) for g in range(4)], axis=0).reshape(H, HP, T)
        dp_, sp_ = nump[:, DH:DH + 1, :], nump[:, DH + 1:DH + 2, :]
        dn_, sn_ = numn[:, DH:DH + 1, :], numn[:, DH + 1:DH + 2, :]
        inv = 1.0 / (dp_ * sn_ + dn_ * sp_ + 1e-6 * (sp_ * sn_))
        oT = (nump * (sn_ * inv) + numn * (sp_ * inv)).reshape(DP, T)
        oT = jnp.where(row == 30, 1.0, oT).astype(bf16)
        h = _tn(xn, w1_v[...]) + b1
        h = jax.nn.gelu(h, approximate=True).astype(bf16)
        yT = _nt(w2T[...], h) + _nn(woT[...], oT)
        out_v[:, pl.ds(r, T)] = (x_v[:, pl.ds(r, T)].astype(f32) + yT).astype(bf16)
        pltpu.make_async_copy(out_v.at[:, pl.ds(r, T)], out_hbm.at[:, pl.ds(r, T)], sem_o.at[i]).start()
        return carry

    lax.fori_loop(0, NTILE, phase2, 0)
    for i in range(NTILE):
        o_copy(i).wait()


@jax.jit
def pallas_parallel_sum__linear_kernel_hedgehog__dense_activation_gelu__prompt_kernel(A_x, A_wqkv, A_w_phi, A_wo, B_x, B_w1, B_b1, B_w2, B_b2):
    xT = A_x.reshape(S, D).T
    hbm = pl.BlockSpec(memory_space=pltpu.MemorySpace.HBM)
    outT = pl.pallas_call(
        _kernel,
        out_shape=jax.ShapeDtypeStruct((D, S), bf16),
        in_specs=[hbm] * 8,
        out_specs=hbm,
        scratch_shapes=[
            pltpu.VMEM((D, S), bf16),
            pltpu.VMEM((D, 3 * D), bf16),
            pltpu.VMEM((DH, H, DH), bf16),
            pltpu.VMEM((D, D), bf16),
            pltpu.VMEM((D, F), bf16),
            pltpu.VMEM((F,), bf16),
            pltpu.VMEM((D, F), bf16),
            pltpu.VMEM((D,), bf16),
            pltpu.VMEM((D, S), bf16),
            pltpu.VMEM((D, S), bf16),
            pltpu.VMEM((DP, D), bf16),
            pltpu.VMEM((DP, D), bf16),
            pltpu.VMEM((DP, D), bf16),
            pltpu.VMEM((D, DP), bf16),
            pltpu.VMEM((576, 128), f32),
            pltpu.VMEM((4, 128, 256), f32),
            pltpu.VMEM((4, 128, 128), bf16),
            pltpu.VMEM((4, 128, 128), bf16),
            pltpu.SemaphoreType.DMA((NTILE,)),
            pltpu.SemaphoreType.DMA((7,)),
            pltpu.SemaphoreType.DMA((NTILE,)),
        ],
        compiler_params=pltpu.CompilerParams(vmem_limit_bytes=64 * 1024 * 1024),
    )(xT, A_wqkv, jnp.transpose(A_w_phi, (1, 0, 2)), A_wo, B_w1, B_b1, B_w2.T, B_b2)
    return outT.T.reshape(1, S, D)
```

```python
import jax
import jax.numpy as jnp
from jax import lax
import jax.experimental.pallas as pl
import jax.experimental.pallas.tpu as pltpu

S, D, H, DH, F = 2048, 448, 16, 28, 1792
NP = H // 2
PR = 2 * DH
T = 256
NTILE = S // T
LOG2E = 1.4426950408889634
f32 = jnp.float32
bf16 = jnp.bfloat16
SCOPES = False


class _Null:
    def __enter__(self): return self
    def __exit__(self, *a): return False


def scope(name):
    return jax.named_scope(name) if SCOPES else _Null()


def _nt(a, b):
    return lax.dot_general(a, b, (((1,), (1,)), ((), ())), preferred_element_type=f32)


def _tn(a, b):
    return lax.dot_general(a, b, (((0,), (0,)), ((), ())), preferred_element_type=f32)


def _nn(a, b):
    return jnp.dot(a, b, preferred_element_type=f32)


def _recip(s):
    r = pl.reciprocal(s, approx=True)
    return r * (2.0 - s * r)


def _pk(x):
    return pltpu.bitcast(x, jnp.uint32)


def _upk(x):
    return pltpu.bitcast(x, bf16)


def _div28(r):
    return (r * 2341) >> 16


def _feature_map(p):
    t = p.shape[-1]
    NP = p.shape[0] // PR
    p3 = p.reshape(NP, PR, t)
    a3 = p3[:, 0:24].reshape(NP, 3, 8, t)
    mid = p3[:, 24:32]
    b3 = p3[:, 32:56].reshape(NP, 3, 8, t)
    low = lax.broadcasted_iota(jnp.int32, (NP, 8, t), 1) < 4
    inf = jnp.float32(jnp.inf)

    def red(op, x3, m, fill, is_a):
        mm = jnp.where(low, m, fill) if is_a else jnp.where(low, fill, m)
        return op(op(x3[:, 0], x3[:, 1]), op(x3[:, 2], mm))

    mxa = jnp.max(red(jnp.maximum, a3, mid, -inf, True), axis=1, keepdims=True)
    mxb = jnp.max(red(jnp.maximum, b3, mid, -inf, False), axis=1, keepdims=True)
    mna = jnp.min(red(jnp.minimum, a3, mid, inf, True), axis=1, keepdims=True)
    mnb = jnp.min(red(jnp.minimum, b3, mid, inf, False), axis=1, keepdims=True)
    outs = []
    for sign in (0, 1):
        if sign == 0:
            ea = jnp.exp2(a3 - mxa[:, None])
            em = jnp.exp2(mid - jnp.where(low, mxa, mxb))
            eb = jnp.exp2(b3 - mxb[:, None])
        else:
            ea = jnp.exp2(mna[:, None] - a3)
            em = jnp.exp2(jnp.where(low, mna, mnb) - mid)
            eb = jnp.exp2(mnb[:, None] - b3)
        sa = jnp.sum(red(jnp.add, ea, em, 0.0, True), axis=1, keepdims=True)
        sb = jnp.sum(red(jnp.add, eb, em, 0.0, False), axis=1, keepdims=True)
        ra = _recip(sa)
        rb = _recip(sb)
        outs.append((ea * ra[:, None]).reshape(NP, 24, t))
        outs.append(em * jnp.where(low, ra, rb))
        outs.append((eb * rb[:, None]).reshape(NP, 24, t))
    outs.append(jnp.zeros((NP, 16, t), f32))
    return jnp.concatenate(outs, axis=1).reshape(NP * 128, t).astype(bf16)


def _kernel(x_hbm, wqkv_hbm, wphi_hbm, wo_hbm, w1_hbm, b1_hbm, w2T_hbm, b2_hbm, out_hbm,
            x_v, wqkv_v, wphi_v, wo_v, w1_v, b1_v, w2T, b2_v, out_v, xn_v,
            wqT, wkT, wvT, woT, b2c, a_pad, kv_acc, kvT, pA, pB, vA, vB, xA, xB, st_m, st_r, zero_s, bdq_s, kv_acc2,
            sem_x, sem_w, sem_o):
    def o_copy(i):
        return pltpu.make_async_copy(out_v.at[:, pl.ds(i * T, T)], out_hbm.at[:, pl.ds(i * T, T)], sem_o.at[i])

    c_x0 = pltpu.make_async_copy(x_hbm.at[:, 0:T], x_v.at[:, 0:T], sem_x.at[0])
    c_x1 = pltpu.make_async_copy(x_hbm.at[:, T:4 * T], x_v.at[:, T:4 * T], sem_x.at[1])
    c_x2 = pltpu.make_async_copy(x_hbm.at[:, 4 * T:S], x_v.at[:, 4 * T:S], sem_x.at[2])
    c_wk = pltpu.make_async_copy(wqkv_hbm.at[:, 384:896], wqkv_v.at[:, 384:896], sem_w.at[0])
    c_wv = pltpu.make_async_copy(wqkv_hbm.at[:, 896:1344], wqkv_v.at[:, 896:1344], sem_w.at[8])
    c_wq = pltpu.make_async_copy(wqkv_hbm.at[:, 0:384], wqkv_v.at[:, 0:384], sem_w.at[7])
    c_w2 = pltpu.make_async_copy(w2T_hbm, w2T, sem_w.at[1])
    c_wo = pltpu.make_async_copy(wo_hbm, wo_v, sem_w.at[2])
    c_w1 = pltpu.make_async_copy(w1_hbm, w1_v, sem_w.at[3])
    c_wphi = pltpu.make_async_copy(wphi_hbm, wphi_v, sem_w.at[4])
    c_b1 = pltpu.make_async_copy(b1_hbm, b1_v, sem_w.at[5])
    c_b2 = pltpu.make_async_copy(b2_hbm, b2_v, sem_w.at[6])

    zero_s[0] = 0
    for c in (c_wphi, c_wk):
        c.start()

    a_pad[...] = jnp.zeros_like(a_pad)
    kv_acc[...] = jnp.zeros_like(kv_acc)
    r1 = lax.broadcasted_iota(jnp.int32, (D, 128), 0)
    c1 = lax.broadcasted_iota(jnp.int32, (D, 128), 1)
    rsel = jnp.where(c1 == r1 - _div28(r1) * DH, 1.0, 0.0).astype(bf16)
    e_r = lax.broadcasted_iota(jnp.int32, (128, 128), 0)
    e_c = lax.broadcasted_iota(jnp.int32, (128, 128), 1)
    eye = jnp.where(e_r == e_c, 1.0, 0.0).astype(bf16)
    c_wphi.wait()
    c_x0.start()
    for d in range(DH):
        a_pad[pl.ds(64 + d, H, stride=DH), 0:DH] = wphi_v[d].astype(f32)

    def win(off, g):
        lo_c = off + 112 * g
        return (lo_c // 128) * 128, ((lo_c + 111) // 128 + 1) * 128

    def bd(off, g):
        c0, c1_ = win(off, g)
        rows = slice(112 * g, 112 * (g + 1))
        t = _nt(rsel[rows], a_pad[64 - off + c0:64 - off + c1_, :].astype(bf16))
        rr = lax.broadcasted_iota(jnp.int32, (112, c1_ - c0), 0)
        cc = lax.broadcasted_iota(jnp.int32, (112, c1_ - c0), 1) + (c0 - off - 112 * g)
        lo = _div28(rr) * DH
        return jnp.where((cc >= lo) & (cc < lo + DH), t, 0.0).astype(bf16)

    def fold(bdg, base, off, dst, gs=range(4)):
        for g in gs:
            c0, c1_ = win(off, g)
            w = _nt(bdg(g), wqkv_v[:, base + c0:base + c1_])
            dst[56 * g:56 * (g + 1), :] = _pk((w * LOG2E).astype(bf16))

    def _off(i):
        return i * T if isinstance(i, int) else pl.multiple_of(i * T, T)

    def stats(i):
        r = _off(i)
        RC = 16
        c0 = x_v[0:RC, pl.ds(r, T)].astype(f32)[0:1]
        s1 = jnp.zeros((8, T), f32)
        s2 = jnp.zeros((8, T), f32)
        for k in range(D // RC):
            d = x_v[RC * k:RC * (k + 1), pl.ds(r, T)].astype(f32) - c0
            d0, d1 = d[0:8], d[8:16]
            s1 = s1 + (d0 + d1)
            s2 = s2 + (d0 * d0 + d1 * d1)
        md = jnp.sum(s1, axis=0, keepdims=True) * (1.0 / D)
        var = jnp.maximum(jnp.sum(s2, axis=0, keepdims=True) * (1.0 / D) - md * md, 0.0)
        st_m[:, pl.ds(r, T)] = jnp.broadcast_to(md + c0, (8, T))
        st_r[:, pl.ds(r, T)] = jnp.broadcast_to(lax.rsqrt(var + 1e-5), (8, T))

    def norm(i):
        r = _off(i)
        x3 = x_v[:, pl.ds(r, T)].astype(f32).reshape(D // 8, 8, T)
        xn = ((x3 - st_m[:, pl.ds(r, T)][None]) * st_r[:, pl.ds(r, T)][None]).reshape(D, T).astype(bf16)
        xn_v[:, pl.ds(r, T)] = _pk(xn)
        return xn

    ones_blk = jnp.where(lax.broadcasted_iota(jnp.int32, (NP, 8, T), 1) < 2, 1.0, 0.0)

    def xn_of(i):
        r = i * T if isinstance(i, int) else pl.multiple_of(i * T, T)
        return _upk(xn_v[:, pl.ds(r, T)])

    def proj(xn, p_dst, v_dst):
        p_dst[...] = _nn(_upk(wkT[...]), xn)
        v3 = _nn(_upk(wvT[...]), xn).reshape(NP, PR, T)
        v_dst[...] = _pk(jnp.concatenate([v3, ones_blk], axis=1).astype(bf16))

    def smkv(p_src, v_src):
        phi = _feature_map(p_src[...])
        for j in range(NP):
            kv_acc[j] += _nt(_upk(v_src[j]), phi[128 * j:128 * (j + 1)])

    ones2 = jnp.where(lax.broadcasted_iota(jnp.int32, (2, 8, T), 1) < 2, 1.0, 0.0)

    def pin(val):
        off = pl.multiple_of(S + zero_s[0], 128)
        x_v[0:16, pl.ds(off, 128)] = val[0:16, 0:128].astype(bf16)

    def step(x_src, p_dst, v_dst, p_src, v_src, i_norm, x_dst, i_stats, last):
        xn = _upk(x_src[...])
        CH = 112
        for c in range(NP):
            g = c % 4
            if c < 4:
                y = _nn(_upk(wkT[56 * g:56 * (g + 1), :]), xn)
                p_dst[112 * g:112 * (g + 1), :] = y
            else:
                y = _nn(_upk(wvT[56 * g:56 * (g + 1), :]), xn)
                v_dst[2 * g:2 * g + 2] = _pk(jnp.concatenate([y.reshape(2, PR, T), ones2], axis=1).astype(bf16))
            phi = _feature_map(p_src[PR * c:PR * (c + 1), :])
            kv_acc[c] += _nt(_upk(v_src[c]), phi)
            if last and c >= 4:
                for jj in (2 * g, 2 * g + 1):
                    phi = _feature_map(p_dst[PR * jj:PR * (jj + 1), :])
                    kv_acc2[jj] = _nt(_upk(v_dst[jj]), phi)
            if c == NP - 1 or (i_norm is None and i_stats is None):
                continue
            pin(y)
            if c < 4 and i_stats is not None:
                rs_ = _off(i_stats)
                if c == 0:
                    c0 = x_v[0:16, pl.ds(rs_, T)].astype(f32)[0:1]
                    s1 = jnp.zeros((8, T), f32)
                    s2 = jnp.zeros((8, T), f32)
                for k in range(7):
                    d = x_v[CH * g + 16 * k:CH * g + 16 * (k + 1), pl.ds(rs_, T)].astype(f32) - c0
                    d0, d1 = d[0:8], d[8:16]
                    s1 = s1 + (d0 + d1)
                    s2 = s2 + (d0 * d0 + d1 * d1)
                if c == 3:
                    md = jnp.sum(s1, axis=0, keepdims=True) * (1.0 / D)
                    var = jnp.maximum(jnp.sum(s2, axis=0, keepdims=True) * (1.0 / D) - md * md, 0.0)
                    st_m[:, pl.ds(rs_, T)] = jnp.broadcast_to(md + c0, (8, T))
                    st_r[:, pl.ds(rs_, T)] = jnp.broadcast_to(lax.rsqrt(var + 1e-5), (8, T))
            if 3 <= c < 7 and i_norm is not None:
                rn = _off(i_norm)
                q = c - 3
                x3 = x_v[CH * q:CH * (q + 1), pl.ds(rn, T)].astype(f32).reshape(CH // 8, 8, T)
                xo = ((x3 - st_m[:, pl.ds(rn, T)][None]) * st_r[:, pl.ds(rn, T)][None]).reshape(CH, T).astype(bf16)
                xn_v[56 * q:56 * (q + 1), pl.ds(rn, T)] = _pk(xo)
                x_dst[56 * q:56 * (q + 1), :] = _pk(xo)

    with scope('bd'):
        bd_k = [bd(64, g) for g in range(4)]
        for g in range(4):
            c0, c1_ = win(0, g)
            bdq_s[56 * g:56 * (g + 1), 0:c1_ - c0] = _pk(bd(0, g))
    with scope('fold_k'):
        c_wk.wait()
        c_wv.start()
        fold(lambda g: bd_k[g], 384, 64, wkT, (0, 1))
    with scope('ln0'):
        c_x0.wait()
        c_x1.start()
        fold(lambda g: bd_k[g], 384, 64, wkT, (2, 3))
        stats(0)
        xn0 = norm(0)
        pA[...] = _nn(_upk(wkT[...]), xn0)
    with scope('fold_v'):
        c_wv.wait()
        c_x2.start()
        for t in range(4):
            n = min(128, D - 128 * t)
            wvT[64 * t:64 * t + n // 2, :] = _pk(_nt(eye[0:n, 0:n], wqkv_v[:, 896 + 128 * t:896 + 128 * t + n]).astype(bf16))
        c_x1.wait()
        for g in range(4):
            y = _nn(_upk(wvT[56 * g:56 * (g + 1), :]), xn0)
            vA[2 * g:2 * g + 2] = _pk(jnp.concatenate([y.reshape(2, PR, T), ones2], axis=1).astype(bf16))
            pin(y)
            if g == 0:
                stats(1)
            if g == 1:
                xB[...] = _pk(norm(1))
            if g == 2:
                stats(2)

    with scope('phase1'):
        bufs = [(xA, pA, vA), (xB, pB, vB)]
        for t in range(1, NTILE):
            if t == 2:
                c_x2.wait()
                for c in (c_wq, c_wo, c_b1, c_b2, c_w1, c_w2):
                    c.start()
            xs, pd, vd = bufs[t % 2]
            xo_, ps, vs = bufs[(t + 1) % 2]
            step(xs, pd, vd, ps, vs, t + 1 if t + 1 < NTILE else None, xo_, t + 2 if t + 2 < NTILE else None, t == NTILE - 1)

    low = lax.broadcasted_iota(jnp.int32, (NP, 8, T), 1) < 4

    def ffn(xn):
        b1 = b1_v[...].astype(f32).reshape(1, F)
        h = _tn(xn, w1_v[...]) + b1
        h = jax.nn.gelu(h, approximate=True).astype(bf16)
        return _nt(w2T[...], h)

    def attn(xn):
        phi = _feature_map(_nn(_upk(wqT[...]), xn))
        num = jnp.concatenate([_nn(_upk(kvT[j]), phi[128 * j:128 * (j + 1)])[None] for j in range(NP)], axis=0)
        ia = _recip(num[:, PR:PR + 1] + 1e-6)
        ib = _recip(num[:, PR + 1:PR + 2] + 1e-6)
        oT = jnp.concatenate([num[:, 0:24] * ia, num[:, 24:32] * jnp.where(low, ia, ib), num[:, 32:56] * ib], axis=1)
        oT = oT.reshape(D, T).astype(bf16)
        return _nn(_upk(woT[...]), oT)

    def finish(i, yT):
        r = _off(i)
        b2t = jnp.concatenate([b2c[...]] * (T // 128), axis=1)
        out_v[:, pl.ds(r, T)] = (x_v[:, pl.ds(r, T)].astype(f32) + b2t + yT).astype(bf16)
        pltpu.make_async_copy(out_v.at[:, pl.ds(r, T)], out_hbm.at[:, pl.ds(r, T)], sem_o.at[i]).start()

    with scope('mid'):
        for c in (c_wq, c_wo, c_b2, c_w1, c_w2, c_b1):
            c.wait()
        fold(lambda g: _upk(bdq_s[56 * g:56 * (g + 1), 0:win(0, g)[1] - win(0, g)[0]]), 0, 0, wqT)
        wo = wo_v[...].astype(f32)
        woT[0:192, :] = _pk(wo[:, 0:384].T.astype(bf16))
        woT[192:224, :] = _pk(jnp.concatenate([wo[:, 384:448], jnp.zeros((D, 64), f32)], axis=1).T[0:64].astype(bf16))
        b2r = jnp.broadcast_to(b2_v[...].astype(f32).reshape(1, D), (128, D))
        b2c[0:384, :] = b2r[:, 0:384].T
        b2c[384:448, :] = jnp.concatenate([b2r[:, 384:448], jnp.zeros((128, 64), f32)], axis=1).T[0:64]

        rd = lax.broadcasted_iota(jnp.int32, (64, 128), 0)
        cf = lax.broadcasted_iota(jnp.int32, (64, 128), 1)
        hd = jnp.where(rd < PR, jnp.where(rd < DH, 0, 1), jnp.where(rd < PR + 2, rd - PR, 2))
        cm = jnp.where(cf < PR, cf, cf - PR)
        hf = jnp.where(cf < 2 * PR, jnp.where(cm < DH, 0, 1), 3)
        own = hd == hf
        for j in range(NP):
            kvT[j] = _pk(jnp.where(own, kv_acc[j] + kv_acc2[j], 0.0).astype(bf16))
        xn_0 = _upk(xn_v[:, 0:T])
        finish(0, ffn(xn_0) + attn(xn_0))

    def phase2(i, carry):
        xn = _upk(xn_v[:, pl.ds(_off(i), T)])
        finish(i, attn(xn) + ffn(xn))
        return carry

    with scope('phase2'):
        lax.fori_loop(1, NTILE, phase2, 0)
    with scope('epilogue'):
        for i in range(NTILE):
            o_copy(i).wait()


@jax.jit
def pallas_parallel_sum__linear_kernel_hedgehog__dense_activation_gelu__prompt_kernel(A_x, A_wqkv, A_w_phi, A_wo, B_x, B_w1, B_b1, B_w2, B_b2):
    xT = A_x.reshape(S, D).T
    hbm = pl.BlockSpec(memory_space=pltpu.MemorySpace.HBM)
    outT = pl.pallas_call(
        _kernel,
        out_shape=jax.ShapeDtypeStruct((D, S), bf16),
        in_specs=[hbm] * 8,
        out_specs=hbm,
        scratch_shapes=[
            pltpu.VMEM((D, S + 128), bf16),
            pltpu.VMEM((D, 3 * D), bf16),
            pltpu.VMEM((DH, H, DH), bf16),
            pltpu.VMEM((D, D), bf16),
            pltpu.VMEM((D, F), bf16),
            pltpu.VMEM((F,), bf16),
            pltpu.VMEM((D, F), bf16),
            pltpu.VMEM((D,), bf16),
            pltpu.VMEM((D, S), bf16),
            pltpu.VMEM((D // 2, S), jnp.uint32),
            pltpu.VMEM((D // 2, D), jnp.uint32),
            pltpu.VMEM((D // 2, D), jnp.uint32),
            pltpu.VMEM((D // 2, D), jnp.uint32),
            pltpu.VMEM((D // 2, D), jnp.uint32),
            pltpu.VMEM((D, 128), f32),
            pltpu.VMEM((576, 128), f32),
            pltpu.VMEM((NP, 64, 128), f32),
            pltpu.VMEM((NP, 32, 128), jnp.uint32),
            pltpu.VMEM((D, T), f32),
            pltpu.VMEM((D, T), f32),
            pltpu.VMEM((NP, 32, T), jnp.uint32),
            pltpu.VMEM((NP, 32, T), jnp.uint32),
            pltpu.VMEM((D // 2, T), jnp.uint32),
            pltpu.VMEM((D // 2, T), jnp.uint32),
            pltpu.VMEM((8, S), f32),
            pltpu.VMEM((8, S), f32),
            pltpu.SMEM((1,), jnp.int32),
            pltpu.VMEM((D // 2, 256), jnp.uint32),
            pltpu.VMEM((NP, 64, 128), f32),
            pltpu.SemaphoreType.DMA((3,)),
            pltpu.SemaphoreType.DMA((9,)),
            pltpu.SemaphoreType.DMA((NTILE,)),
        ],
        compiler_params=pltpu.CompilerParams(vmem_limit_bytes=64 * 1024 * 1024),
    )(xT, A_wqkv, jnp.transpose(A_w_phi, (1, 0, 2)), A_wo, B_w1, B_b1, B_w2.T, B_b2)
    return outT.T.reshape(1, S, D)
```

```python
import jax
import jax.numpy as jnp
from jax import lax
import jax.experimental.pallas as pl
import jax.experimental.pallas.tpu as pltpu

S, D, H, DH, F = 2048, 448, 16, 28, 1792
NP = H // 2
PR = 2 * DH
G = 4 * DH
T = 256
NTILE = S // T
LOG2E = 1.4426950408889634
f32 = jnp.float32
bf16 = jnp.bfloat16
u32 = jnp.uint32


def _nt(a, b):
    return lax.dot_general(a, b, (((1,), (1,)), ((), ())), preferred_element_type=f32)


def _tn(a, b):
    return lax.dot_general(a, b, (((0,), (0,)), ((), ())), preferred_element_type=f32)


def _nn(a, b):
    return jnp.dot(a, b, preferred_element_type=f32)


def _recip(s):
    r = pl.reciprocal(s, approx=True)
    return r * (2.0 - s * r)


def _pk(x):
    return pltpu.bitcast(x, u32)


def _upk(x):
    return pltpu.bitcast(x, bf16)


def _div28(r):
    return (r * 2341) >> 16


def _feature_map(p):
    t = p.shape[-1]
    n = p.shape[0] // PR
    p3 = p.reshape(n, PR, t)
    a3 = p3[:, 0:24].reshape(n, 3, 8, t)
    mid = p3[:, 24:32]
    b3 = p3[:, 32:56].reshape(n, 3, 8, t)
    low = lax.broadcasted_iota(jnp.int32, (n, 8, t), 1) < 4
    inf = jnp.float32(jnp.inf)

    def red(op, x3, m, fill, is_a):
        mm = jnp.where(low, m, fill) if is_a else jnp.where(low, fill, m)
        return op(op(x3[:, 0], x3[:, 1]), op(x3[:, 2], mm))

    mxa = jnp.max(red(jnp.maximum, a3, mid, -inf, True), axis=1, keepdims=True)
    mxb = jnp.max(red(jnp.maximum, b3, mid, -inf, False), axis=1, keepdims=True)
    mna = jnp.min(red(jnp.minimum, a3, mid, inf, True), axis=1, keepdims=True)
    mnb = jnp.min(red(jnp.minimum, b3, mid, inf, False), axis=1, keepdims=True)
    outs = []
    for sign in (0, 1):
        if sign == 0:
            ea = jnp.exp2(a3 - mxa[:, None])
            em = jnp.exp2(mid - jnp.where(low, mxa, mxb))
            eb = jnp.exp2(b3 - mxb[:, None])
        else:
            ea = jnp.exp2(mna[:, None] - a3)
            em = jnp.exp2(jnp.where(low, mna, mnb) - mid)
            eb = jnp.exp2(mnb[:, None] - b3)
        ra = _recip(jnp.sum(red(jnp.add, ea, em, 0.0, True), axis=1, keepdims=True))
        rb = _recip(jnp.sum(red(jnp.add, eb, em, 0.0, False), axis=1, keepdims=True))
        outs.append((ea * ra[:, None]).reshape(n, 24, t))
        outs.append(em * jnp.where(low, ra, rb))
        outs.append((eb * rb[:, None]).reshape(n, 24, t))
    outs.append(jnp.zeros((n, 16, t), f32))
    return jnp.concatenate(outs, axis=1).reshape(n * 128, t).astype(bf16)


def _kernel(x_hbm, wqkv_hbm, wphi_hbm, wo_hbm, w1_hbm, b1_hbm, w2T_hbm, b2_hbm, out_hbm,
            x_v, wqkv_v, wphi_v, wo_v, w1_v, b1_v, w2T, b2_v, out_v, xn_v,
            wqT, wkT, wvT, woT, b2c, a_pad, bdq_s, kv_acc, kvT,
            pA, pB, vA, vB, xA, xB, st_m, st_r,
            sem_x, sem_w, sem_o):
    cp = pltpu.make_async_copy
    c_x0 = cp(x_hbm.at[:, 0:T], x_v.at[:, 0:T], sem_x.at[0])
    c_x1 = cp(x_hbm.at[:, T:4 * T], x_v.at[:, T:4 * T], sem_x.at[1])
    c_x2 = cp(x_hbm.at[:, 4 * T:S], x_v.at[:, 4 * T:S], sem_x.at[2])
    c_wk = cp(wqkv_hbm.at[:, 384:896], wqkv_v.at[:, 384:896], sem_w.at[0])
    c_wv = cp(wqkv_hbm.at[:, 896:1344], wqkv_v.at[:, 896:1344], sem_w.at[1])
    c_wq = cp(wqkv_hbm.at[:, 0:384], wqkv_v.at[:, 0:384], sem_w.at[2])
    c_wphi = cp(wphi_hbm, wphi_v, sem_w.at[3])
    c_late = [c_wq,
              cp(wo_hbm, wo_v, sem_w.at[4]), cp(b1_hbm, b1_v, sem_w.at[5]), cp(b2_hbm, b2_v, sem_w.at[6]),
              cp(w1_hbm, w1_v, sem_w.at[7]), cp(w2T_hbm, w2T, sem_w.at[8])]

    def o_copy(i, r):
        return cp(out_v.at[:, pl.ds(r, T)], out_hbm.at[:, pl.ds(r, T)], sem_o.at[i])

    c_wphi.start()
    c_wk.start()

    a_pad[...] = jnp.zeros_like(a_pad)
    kv_acc[...] = jnp.zeros_like(kv_acc)
    r1 = lax.broadcasted_iota(jnp.int32, (D, 128), 0)
    c1 = lax.broadcasted_iota(jnp.int32, (D, 128), 1)
    rsel = jnp.where(c1 == r1 - _div28(r1) * DH, 1.0, 0.0).astype(bf16)
    eye = jnp.where(lax.broadcasted_iota(jnp.int32, (128, 128), 0)
                    == lax.broadcasted_iota(jnp.int32, (128, 128), 1), 1.0, 0.0).astype(bf16)
    c_wphi.wait()
    c_x0.start()
    for d in range(DH):
        a_pad[pl.ds(64 + d, H, stride=DH), 0:DH] = wphi_v[d].astype(f32)

    def win(off, g):
        lo_c = off + G * g
        return (lo_c // 128) * 128, ((lo_c + G - 1) // 128 + 1) * 128

    def bd(off, g):
        c0, c1_ = win(off, g)
        t = _nt(rsel[G * g:G * (g + 1)], a_pad[64 - off + c0:64 - off + c1_, :].astype(bf16))
        rr = lax.broadcasted_iota(jnp.int32, (G, c1_ - c0), 0)
        cc = lax.broadcasted_iota(jnp.int32, (G, c1_ - c0), 1) + (c0 - off - G * g)
        lo = _div28(rr) * DH
        return jnp.where((cc >= lo) & (cc < lo + DH), t, 0.0).astype(bf16)

    def fold(bdg, base, off, dst, gs):
        for g in gs:
            c0, c1_ = win(off, g)
            w = _nt(bdg(g), wqkv_v[:, base + c0:base + c1_])
            dst[PR * g:PR * (g + 1), :] = _pk((w * LOG2E).astype(bf16))

    def stat_init(r):
        return x_v[0:16, r:r + T].astype(f32)[0:1], jnp.zeros((8, T), f32), jnp.zeros((8, T), f32)

    def stat_acc(r, rows, st):
        c0, s1, s2 = st
        for k in range(rows.start, rows.stop, 16):
            d = x_v[k:k + 16, r:r + T].astype(f32) - c0
            d0, d1 = d[0:8], d[8:16]
            s1 = s1 + (d0 + d1)
            s2 = s2 + (d0 * d0 + d1 * d1)
        return c0, s1, s2

    def stat_fin(r, st):
        c0, s1, s2 = st
        md = jnp.sum(s1, axis=0, keepdims=True) * (1.0 / D)
        var = jnp.maximum(jnp.sum(s2, axis=0, keepdims=True) * (1.0 / D) - md * md, 0.0)
        st_m[:, r:r + T] = jnp.broadcast_to(md + c0, (8, T))
        st_r[:, r:r + T] = jnp.broadcast_to(lax.rsqrt(var + 1e-5), (8, T))

    def stats(t):
        stat_fin(t * T, stat_acc(t * T, slice(0, D), stat_init(t * T)))

    def norm(t, rows=slice(0, D)):
        r, n = t * T, rows.stop - rows.start
        x3 = x_v[rows, r:r + T].astype(f32).reshape(n // 8, 8, T)
        xn = ((x3 - st_m[:, r:r + T][None]) * st_r[:, r:r + T][None]).reshape(n, T).astype(bf16)
        xn_v[rows.start // 2:rows.stop // 2, r:r + T] = _pk(xn)
        return xn

    ones2 = jnp.where(lax.broadcasted_iota(jnp.int32, (2, 8, T), 1) < 2, 1.0, 0.0)

    def vproj(g, xn, v_dst):
        y = _nn(_upk(wvT[PR * g:PR * (g + 1), :]), xn).reshape(2, PR, T)
        v_dst[2 * g:2 * g + 2] = _pk(jnp.concatenate([y, ones2], axis=1).astype(bf16))

    def smkv(j, p_src, v_src):
        kv_acc[j] += _nt(_upk(v_src[j]), _feature_map(p_src[PR * j:PR * (j + 1), :]))

    def step(t, x_src, p_dst, v_dst, x_dst, p_src, v_src):
        xn = _upk(x_src[...])
        st = None
        for c in range(NP):
            g = c % 4
            if c < 4:
                p_dst[G * g:G * (g + 1), :] = _nn(_upk(wkT[PR * g:PR * (g + 1), :]), xn)
            else:
                vproj(g, xn, v_dst)
            smkv(c, p_src, v_src)
            if c < 4 and t + 2 < NTILE:
                r = (t + 2) * T
                st = stat_acc(r, slice(G * g, G * (g + 1)), stat_init(r) if c == 0 else st)
                if c == 3:
                    stat_fin(r, st)
            if 3 <= c < 7 and t + 1 < NTILE:
                q = c - 3
                x_dst[PR * q:PR * (q + 1), :] = _pk(norm(t + 1, slice(G * q, G * (q + 1))))

    bd_k = [bd(64, g) for g in range(4)]
    for g in range(4):
        c0, c1_ = win(0, g)
        bdq_s[PR * g:PR * (g + 1), 0:c1_ - c0] = _pk(bd(0, g))
    c_wk.wait()
    c_wv.start()
    fold(lambda g: bd_k[g], 384, 64, wkT, (0, 1))
    c_x0.wait()
    c_x1.start()
    fold(lambda g: bd_k[g], 384, 64, wkT, (2, 3))
    stats(0)
    xn0 = norm(0)
    pA[...] = _nn(_upk(wkT[...]), xn0)
    c_wv.wait()
    c_x2.start()
    for t in range(4):
        n = min(128, D - 128 * t)
        wvT[64 * t:64 * t + n // 2, :] = _pk(
            _nt(eye[0:n, 0:n], wqkv_v[:, 896 + 128 * t:896 + 128 * t + n]).astype(bf16))
    c_x1.wait()
    for g in range(4):
        vproj(g, xn0, vA)
        if g == 0:
            stats(1)
        if g == 1:
            xB[...] = _pk(norm(1))
        if g == 2:
            stats(2)

    bufs = ((xA, pA, vA), (xB, pB, vB))
    for t in range(1, NTILE):
        if t == 2:
            c_x2.wait()
            for c in c_late:
                c.start()
        step(t, *bufs[t % 2][:3], *bufs[(t + 1) % 2][:3])

    low = lax.broadcasted_iota(jnp.int32, (NP, 8, T), 1) < 4

    def hidden(xn, cs):
        b1 = b1_v[...].astype(f32).reshape(1, F)
        return jax.nn.gelu(_tn(xn, w1_v[:, cs]) + b1[:, cs], approximate=True).astype(bf16)

    def attn(xn):
        phi = _feature_map(_nn(_upk(wqT[...]), xn))
        num = jnp.concatenate([_nn(_upk(kvT[j]), phi[128 * j:128 * (j + 1)])[None] for j in range(NP)], axis=0)
        ia = _recip(num[:, PR:PR + 1] + 1e-6)
        ib = _recip(num[:, PR + 1:PR + 2] + 1e-6)
        oT = jnp.concatenate([num[:, 0:24] * ia, num[:, 24:32] * jnp.where(low, ia, ib), num[:, 32:56] * ib], axis=1)
        return _nn(_upk(woT[...]), oT.reshape(D, T).astype(bf16))

    def finish(i, r, yT):
        b2t = jnp.concatenate([b2c[...]] * (T // 128), axis=1)
        out_v[:, pl.ds(r, T)] = (x_v[:, pl.ds(r, T)].astype(f32) + b2t + yT).astype(bf16)
        o_copy(i, r).start()

    for c in c_late:
        c.wait()
    xn_0 = _upk(xn_v[:, 0:T])

    def bdq(g):
        c0, c1_ = win(0, g)
        return _upk(bdq_s[PR * g:PR * (g + 1), 0:c1_ - c0])

    fold(bdq, 0, 0, wqT, (0, 1))
    hs = []
    for c in range(NP):
        if c < 7:
            hs.append(hidden(xn_0, slice(256 * c, 256 * (c + 1))))
        smkv(c, pB, vB)
        if c < 2:
            fold(bdq, 0, 0, wqT, (c + 2,))
    wo = wo_v[...].astype(f32)
    woT[0:192, :] = _pk(wo[:, 0:384].T.astype(bf16))
    woT[192:224, :] = _pk(jnp.concatenate([wo[:, 384:448], jnp.zeros((D, 64), f32)], axis=1).T[0:64].astype(bf16))
    b2r = jnp.broadcast_to(b2_v[...].astype(f32).reshape(1, D), (128, D))
    b2c[0:384, :] = b2r[:, 0:384].T
    b2c[384:448, :] = jnp.concatenate([b2r[:, 384:448], jnp.zeros((128, 64), f32)], axis=1).T[0:64]
    rd = lax.broadcasted_iota(jnp.int32, (64, 128), 0)
    cf = lax.broadcasted_iota(jnp.int32, (64, 128), 1)
    hd = jnp.where(rd < PR, jnp.where(rd < DH, 0, 1), jnp.where(rd < PR + 2, rd - PR, 2))
    cm = jnp.where(cf < PR, cf, cf - PR)
    hf = jnp.where(cf < 2 * PR, jnp.where(cm < DH, 0, 1), 3)
    own = hd == hf
    for j in range(NP):
        kvT[j] = _pk(jnp.where(own, kv_acc[j], 0.0).astype(bf16))
    finish(0, 0, attn(xn_0) + _nt(w2T[...], jnp.concatenate(hs, axis=1)))

    def phase2(i, carry):
        r = pl.multiple_of(i * T, T)
        xn = _upk(xn_v[:, pl.ds(r, T)])
        finish(i, r, attn(xn) + _nt(w2T[...], hidden(xn, slice(0, F))))
        return carry

    lax.fori_loop(1, NTILE, phase2, 0)
    for i in range(NTILE):
        o_copy(i, i * T).wait()


@jax.jit
def pallas_parallel_sum__linear_kernel_hedgehog__dense_activation_gelu__prompt_kernel(
    A_x: jax.Array,
    A_wqkv: jax.Array,
    A_w_phi: jax.Array,
    A_wo: jax.Array,
    B_x: jax.Array,
    B_w1: jax.Array,
    B_b1: jax.Array,
    B_w2: jax.Array,
    B_b2: jax.Array,
):
    hbm = pl.BlockSpec(memory_space=pltpu.MemorySpace.HBM)
    outT = pl.pallas_call(
        _kernel,
        out_shape=jax.ShapeDtypeStruct((D, S), bf16),
        in_specs=[hbm] * 8,
        out_specs=hbm,
        scratch_shapes=[
            pltpu.VMEM((D, S), bf16),
            pltpu.VMEM((D, 3 * D), bf16),
            pltpu.VMEM((DH, H, DH), bf16),
            pltpu.VMEM((D, D), bf16),
            pltpu.VMEM((D, F), bf16),
            pltpu.VMEM((F,), bf16),
            pltpu.VMEM((D, F), bf16),
            pltpu.VMEM((D,), bf16),
            pltpu.VMEM((D, S), bf16),
            pltpu.VMEM((D // 2, S), u32),
            pltpu.VMEM((D // 2, D), u32),
            pltpu.VMEM((D // 2, D), u32),
            pltpu.VMEM((D // 2, D), u32),
            pltpu.VMEM((D // 2, D), u32),
            pltpu.VMEM((D, 128), f32),
            pltpu.VMEM((576, 128), f32),
            pltpu.VMEM((D // 2, 256), u32),
            pltpu.VMEM((NP, 64, 128), f32),
            pltpu.VMEM((NP, 32, 128), u32),
            pltpu.VMEM((D, T), f32),
            pltpu.VMEM((D, T), f32),
            pltpu.VMEM((NP, 32, T), u32),
            pltpu.VMEM((NP, 32, T), u32),
            pltpu.VMEM((D // 2, T), u32),
            pltpu.VMEM((D // 2, T), u32),
            pltpu.VMEM((8, S), f32),
            pltpu.VMEM((8, S), f32),
            pltpu.SemaphoreType.DMA((3,)),
            pltpu.SemaphoreType.DMA((9,)),
            pltpu.SemaphoreType.DMA((NTILE,)),
        ],
        compiler_params=pltpu.CompilerParams(vmem_limit_bytes=64 * 1024 * 1024),
    )(A_x.reshape(S, D).T, A_wqkv, jnp.transpose(A_w_phi, (1, 0, 2)), A_wo, B_w1, B_b1, B_w2.T, B_b2)
    return outT.T.reshape(1, S, D)
```

```python
import jax
import jax.numpy as jnp
from jax import lax
import jax.experimental.pallas as pl
import jax.experimental.pallas.tpu as pltpu

S, D, H, DH, F = 2048, 448, 16, 28, 1792
NP = H // 2
PR = 2 * DH
G = 4 * DH
T = 256
NTILE = S // T
LOG2E = 1.4426950408889634
f32 = jnp.float32
bf16 = jnp.bfloat16
u32 = jnp.uint32


def _nt(a, b):
    return lax.dot_general(a, b, (((1,), (1,)), ((), ())), preferred_element_type=f32)


def _tn(a, b):
    return lax.dot_general(a, b, (((0,), (0,)), ((), ())), preferred_element_type=f32)


def _nn(a, b):
    return jnp.dot(a, b, preferred_element_type=f32)


def _recip(s):
    r = pl.reciprocal(s, approx=True)
    return r * (2.0 - s * r)


def _pk(x):
    return pltpu.bitcast(x, u32)


def _upk(x):
    return pltpu.bitcast(x, bf16)


def _div28(r):
    return (r * 2341) >> 16


def _feature_map(p):
    t = p.shape[-1]
    n = p.shape[0] // PR
    p3 = p.reshape(n, PR, t)
    a3 = p3[:, 0:24].reshape(n, 3, 8, t)
    mid = p3[:, 24:32]
    b3 = p3[:, 32:56].reshape(n, 3, 8, t)
    low = lax.broadcasted_iota(jnp.int32, (n, 8, t), 1) < 4
    inf = jnp.float32(jnp.inf)

    def red(op, x3, m, fill, is_a):
        mm = jnp.where(low, m, fill) if is_a else jnp.where(low, fill, m)
        return op(op(x3[:, 0], x3[:, 1]), op(x3[:, 2], mm))

    mxa = jnp.max(red(jnp.maximum, a3, mid, -inf, True), axis=1, keepdims=True)
    mxb = jnp.max(red(jnp.maximum, b3, mid, -inf, False), axis=1, keepdims=True)
    mna = jnp.min(red(jnp.minimum, a3, mid, inf, True), axis=1, keepdims=True)
    mnb = jnp.min(red(jnp.minimum, b3, mid, inf, False), axis=1, keepdims=True)
    outs = []
    for sign in (0, 1):
        if sign == 0:
            ea = jnp.exp2(a3 - mxa[:, None])
            em = jnp.exp2(mid - jnp.where(low, mxa, mxb))
            eb = jnp.exp2(b3 - mxb[:, None])
        else:
            ea = jnp.exp2(mna[:, None] - a3)
            em = jnp.exp2(jnp.where(low, mna, mnb) - mid)
            eb = jnp.exp2(mnb[:, None] - b3)
        ra = _recip(jnp.sum(red(jnp.add, ea, em, 0.0, True), axis=1, keepdims=True))
        rb = _recip(jnp.sum(red(jnp.add, eb, em, 0.0, False), axis=1, keepdims=True))
        outs.append((ea * ra[:, None]).reshape(n, 24, t))
        outs.append(em * jnp.where(low, ra, rb))
        outs.append((eb * rb[:, None]).reshape(n, 24, t))
    outs.append(jnp.zeros((n, 16, t), f32))
    return jnp.concatenate(outs, axis=1).reshape(n * 128, t).astype(bf16)


def _kernel(x_hbm, wqkv_hbm, wphi_hbm, wo_hbm, w1_hbm, b1_hbm, w2T_hbm, b2_hbm, out_hbm,
            x_v, wqkv_v, wphi_v, wo_v, w1_v, b1_v, w2T, b2_v, out_v, xn_v,
            wqT, wkT, wvT, woT, b2c, a_pad, bdq_s, kv_acc, kvT,
            pA, pB, vA, vB, xA, xB, st_m, st_r,
            sem_x, sem_w, sem_o):
    cp = pltpu.make_async_copy
    c_x0 = cp(x_hbm.at[:, 0:T], x_v.at[:, 0:T], sem_x.at[0])
    c_x1 = cp(x_hbm.at[:, T:4 * T], x_v.at[:, T:4 * T], sem_x.at[1])
    c_x2 = cp(x_hbm.at[:, 4 * T:S], x_v.at[:, 4 * T:S], sem_x.at[2])
    c_wk = cp(wqkv_hbm.at[:, 384:896], wqkv_v.at[:, 384:896], sem_w.at[0])
    c_wv = cp(wqkv_hbm.at[:, 896:1344], wqkv_v.at[:, 896:1344], sem_w.at[1])
    c_wq = cp(wqkv_hbm.at[:, 0:384], wqkv_v.at[:, 0:384], sem_w.at[2])
    c_wphi = cp(wphi_hbm, wphi_v, sem_w.at[3])
    c_late = [c_wq,
              cp(wo_hbm, wo_v, sem_w.at[4]), cp(b1_hbm, b1_v, sem_w.at[5]), cp(b2_hbm, b2_v, sem_w.at[6]),
              cp(w1_hbm, w1_v, sem_w.at[7]), cp(w2T_hbm, w2T, sem_w.at[8])]

    def o_copy(i, r, w):
        return cp(out_v.at[:, pl.ds(r, w)], out_hbm.at[:, pl.ds(r, w)], sem_o.at[i])

    c_wphi.start()
    c_wk.start()

    a_pad[...] = jnp.zeros_like(a_pad)
    kv_acc[...] = jnp.zeros_like(kv_acc)
    r1 = lax.broadcasted_iota(jnp.int32, (D, 128), 0)
    c1 = lax.broadcasted_iota(jnp.int32, (D, 128), 1)
    rsel = jnp.where(c1 == r1 - _div28(r1) * DH, 1.0, 0.0).astype(bf16)
    eye = jnp.where(lax.broadcasted_iota(jnp.int32, (128, 128), 0)
                    == lax.broadcasted_iota(jnp.int32, (128, 128), 1), 1.0, 0.0).astype(bf16)
    c_wphi.wait()
    c_x0.start()
    for d in range(DH):
        a_pad[pl.ds(64 + d, H, stride=DH), 0:DH] = wphi_v[d].astype(f32)

    def win(off, g):
        lo_c = off + G * g
        return (lo_c // 128) * 128, ((lo_c + G - 1) // 128 + 1) * 128

    def bd(off, g):
        c0, c1_ = win(off, g)
        t = _nt(rsel[G * g:G * (g + 1)], a_pad[64 - off + c0:64 - off + c1_, :].astype(bf16))
        rr = lax.broadcasted_iota(jnp.int32, (G, c1_ - c0), 0)
        cc = lax.broadcasted_iota(jnp.int32, (G, c1_ - c0), 1) + (c0 - off - G * g)
        lo = _div28(rr) * DH
        return jnp.where((cc >= lo) & (cc < lo + DH), t, 0.0).astype(bf16)

    def fold(bdg, base, off, dst, gs):
        for g in gs:
            c0, c1_ = win(off, g)
            w = _nt(bdg(g), wqkv_v[:, base + c0:base + c1_])
            dst[PR * g:PR * (g + 1), :] = _pk((w * LOG2E).astype(bf16))

    def stat_init(r):
        return x_v[0:16, r:r + T].astype(f32)[0:1], jnp.zeros((8, T), f32), jnp.zeros((8, T), f32)

    def stat_acc(r, rows, st):
        c0, s1, s2 = st
        for k in range(rows.start, rows.stop, 16):
            d = x_v[k:k + 16, r:r + T].astype(f32) - c0
            d0, d1 = d[0:8], d[8:16]
            s1 = s1 + (d0 + d1)
            s2 = s2 + (d0 * d0 + d1 * d1)
        return c0, s1, s2

    def stat_fin(r, st):
        c0, s1, s2 = st
        md = jnp.sum(s1, axis=0, keepdims=True) * (1.0 / D)
        var = jnp.maximum(jnp.sum(s2, axis=0, keepdims=True) * (1.0 / D) - md * md, 0.0)
        st_m[:, r:r + T] = jnp.broadcast_to(md + c0, (8, T))
        st_r[:, r:r + T] = jnp.broadcast_to(lax.rsqrt(var + 1e-5), (8, T))

    def stats(t):
        stat_fin(t * T, stat_acc(t * T, slice(0, D), stat_init(t * T)))

    def norm(t, rows=slice(0, D)):
        r, n = t * T, rows.stop - rows.start
        x3 = x_v[rows, r:r + T].astype(f32).reshape(n // 8, 8, T)
        xn = ((x3 - st_m[:, r:r + T][None]) * st_r[:, r:r + T][None]).reshape(n, T).astype(bf16)
        xn_v[rows.start // 2:rows.stop // 2, r:r + T] = _pk(xn)
        return xn

    ones2 = jnp.where(lax.broadcasted_iota(jnp.int32, (2, 8, T), 1) < 2, 1.0, 0.0)

    def vproj(g, xn, v_dst):
        y = _nn(_upk(wvT[PR * g:PR * (g + 1), :]), xn).reshape(2, PR, T)
        v_dst[2 * g:2 * g + 2] = _pk(jnp.concatenate([y, ones2], axis=1).astype(bf16))

    def smkv(j, p_src, v_src):
        kv_acc[j] += _nt(_upk(v_src[j]), _feature_map(p_src[PR * j:PR * (j + 1), :]))

    def step(t, x_src, p_dst, v_dst, x_dst, p_src, v_src):
        xn = _upk(x_src[...])
        st = None
        for c in range(NP):
            g = c % 4
            if c < 4:
                p_dst[G * g:G * (g + 1), :] = _nn(_upk(wkT[PR * g:PR * (g + 1), :]), xn)
            else:
                vproj(g, xn, v_dst)
            smkv(c, p_src, v_src)
            if c < 4 and t + 2 < NTILE:
                r = (t + 2) * T
                st = stat_acc(r, slice(G * g, G * (g + 1)), stat_init(r) if c == 0 else st)
                if c == 3:
                    stat_fin(r, st)
            if 3 <= c < 7 and t + 1 < NTILE:
                q = c - 3
                x_dst[PR * q:PR * (q + 1), :] = _pk(norm(t + 1, slice(G * q, G * (q + 1))))

    bd_k = [bd(64, g) for g in range(4)]
    for g in range(4):
        c0, c1_ = win(0, g)
        bdq_s[PR * g:PR * (g + 1), 0:c1_ - c0] = _pk(bd(0, g))
    c_wk.wait()
    c_wv.start()
    fold(lambda g: bd_k[g], 384, 64, wkT, (0, 1))
    c_x0.wait()
    c_x1.start()
    fold(lambda g: bd_k[g], 384, 64, wkT, (2, 3))
    stats(0)
    xn0 = norm(0)
    pA[...] = _nn(_upk(wkT[...]), xn0)
    c_wv.wait()
    c_x2.start()
    for t in range(4):
        n = min(128, D - 128 * t)
        wvT[64 * t:64 * t + n // 2, :] = _pk(
            _nt(eye[0:n, 0:n], wqkv_v[:, 896 + 128 * t:896 + 128 * t + n]).astype(bf16))
    c_x1.wait()
    for g in range(4):
        vproj(g, xn0, vA)
        if g == 0:
            stats(1)
        if g == 1:
            xB[...] = _pk(norm(1))
        if g == 2:
            stats(2)

    bufs = ((xA, pA, vA), (xB, pB, vB))
    for t in range(1, NTILE):
        if t == 2:
            c_x2.wait()
            for c in c_late:
                c.start()
        step(t, *bufs[t % 2][:3], *bufs[(t + 1) % 2][:3])

    def hidden(xn, cs):
        b1 = b1_v[...].astype(f32).reshape(1, F)
        return jax.nn.gelu(_tn(xn, w1_v[:, cs]) + b1[:, cs], approximate=True).astype(bf16)

    def attn_o(xn):
        w = xn.shape[1]
        low = lax.broadcasted_iota(jnp.int32, (NP, 8, w), 1) < 4
        phi = _feature_map(_nn(_upk(wqT[...]), xn))
        num = jnp.concatenate([_nn(_upk(kvT[j]), phi[128 * j:128 * (j + 1)])[None] for j in range(NP)], axis=0)
        ia = _recip(num[:, PR:PR + 1] + 1e-6)
        ib = _recip(num[:, PR + 1:PR + 2] + 1e-6)
        oT = jnp.concatenate([num[:, 0:24] * ia, num[:, 24:32] * jnp.where(low, ia, ib), num[:, 32:56] * ib], axis=1)
        return oT.reshape(D, w).astype(bf16)

    def attn(xn):
        return _nn(_upk(woT[...]), attn_o(xn))

    def finish(i, r, yT):
        w = yT.shape[1]
        b2t = jnp.concatenate([b2c[...]] * (w // 128), axis=1)
        out_v[:, pl.ds(r, w)] = (x_v[:, pl.ds(r, w)].astype(f32) + b2t + yT).astype(bf16)
        o_copy(i, r, w).start()

    for c in c_late:
        c.wait()
    xn_0 = _upk(xn_v[:, 0:T])

    def bdq(g):
        c0, c1_ = win(0, g)
        return _upk(bdq_s[PR * g:PR * (g + 1), 0:c1_ - c0])

    fold(bdq, 0, 0, wqT, (0, 1))
    hs = []
    for c in range(NP):
        if c < 7:
            hs.append(hidden(xn_0, slice(256 * c, 256 * (c + 1))))
        smkv(c, pB, vB)
        if c < 2:
            fold(bdq, 0, 0, wqT, (c + 2,))
    wo = wo_v[...].astype(f32)
    woT[0:192, :] = _pk(wo[:, 0:384].T.astype(bf16))
    woT[192:224, :] = _pk(jnp.concatenate([wo[:, 384:448], jnp.zeros((D, 64), f32)], axis=1).T[0:64].astype(bf16))
    b2r = jnp.broadcast_to(b2_v[...].astype(f32).reshape(1, D), (128, D))
    b2c[0:384, :] = b2r[:, 0:384].T
    b2c[384:448, :] = jnp.concatenate([b2r[:, 384:448], jnp.zeros((128, 64), f32)], axis=1).T[0:64]
    rd = lax.broadcasted_iota(jnp.int32, (64, 128), 0)
    cf = lax.broadcasted_iota(jnp.int32, (64, 128), 1)
    hd = jnp.where(rd < PR, jnp.where(rd < DH, 0, 1), jnp.where(rd < PR + 2, rd - PR, 2))
    cm = jnp.where(cf < PR, cf, cf - PR)
    hf = jnp.where(cf < 2 * PR, jnp.where(cm < DH, 0, 1), 3)
    own = hd == hf
    for j in range(NP):
        kvT[j] = _pk(jnp.where(own, kv_acc[j], 0.0).astype(bf16))
    finish(0, 0, attn(xn_0) + _nt(w2T[...], jnp.concatenate(hs, axis=1)))

    def tile(i, r, w):
        xn = _upk(xn_v[:, pl.ds(r, w)])
        finish(i, r, attn(xn) + _nt(w2T[...], hidden(xn, slice(0, F))))

    def phase2(i, carry):
        tile(i + 1, pl.multiple_of(T + i * 2 * T, T), 2 * T)
        return carry

    lax.fori_loop(0, 3, phase2, 0)
    r = S - T
    xn = _upk(xn_v[:, r:S])
    oT = attn_o(xn)
    h = hidden(xn, slice(0, F))
    halves = []
    for m in range(2):
        rows = slice(224 * m, 224 * (m + 1))
        yT = _nn(_upk(woT[112 * m:112 * (m + 1), :]), oT) + _nt(w2T[rows, :], h)
        b2t = jnp.concatenate([b2c[rows, :]] * (T // 128), axis=1)
        out_v[rows, r:S] = (x_v[rows, r:S].astype(f32) + b2t + yT).astype(bf16)
        halves.append(cp(out_v.at[rows, r:S], out_hbm.at[rows, r:S], sem_o.at[4 + m]))
        halves[-1].start()
    o_copy(0, 0, T).wait()
    for i in range(3):
        o_copy(i + 1, T + i * 2 * T, 2 * T).wait()
    for c in halves:
        c.wait()


@jax.jit
def pallas_parallel_sum__linear_kernel_hedgehog__dense_activation_gelu__prompt_kernel(
    A_x: jax.Array,
    A_wqkv: jax.Array,
    A_w_phi: jax.Array,
    A_wo: jax.Array,
    B_x: jax.Array,
    B_w1: jax.Array,
    B_b1: jax.Array,
    B_w2: jax.Array,
    B_b2: jax.Array,
):
    hbm = pl.BlockSpec(memory_space=pltpu.MemorySpace.HBM)
    outT = pl.pallas_call(
        _kernel,
        out_shape=jax.ShapeDtypeStruct((D, S), bf16),
        in_specs=[hbm] * 8,
        out_specs=hbm,
        scratch_shapes=[
            pltpu.VMEM((D, S), bf16),
            pltpu.VMEM((D, 3 * D), bf16),
            pltpu.VMEM((DH, H, DH), bf16),
            pltpu.VMEM((D, D), bf16),
            pltpu.VMEM((D, F), bf16),
            pltpu.VMEM((F,), bf16),
            pltpu.VMEM((D, F), bf16),
            pltpu.VMEM((D,), bf16),
            pltpu.VMEM((D, S), bf16),
            pltpu.VMEM((D // 2, S), u32),
            pltpu.VMEM((D // 2, D), u32),
            pltpu.VMEM((D // 2, D), u32),
            pltpu.VMEM((D // 2, D), u32),
            pltpu.VMEM((D // 2, D), u32),
            pltpu.VMEM((D, 128), f32),
            pltpu.VMEM((576, 128), f32),
            pltpu.VMEM((D // 2, 256), u32),
            pltpu.VMEM((NP, 64, 128), f32),
            pltpu.VMEM((NP, 32, 128), u32),
            pltpu.VMEM((D, T), f32),
            pltpu.VMEM((D, T), f32),
            pltpu.VMEM((NP, 32, T), u32),
            pltpu.VMEM((NP, 32, T), u32),
            pltpu.VMEM((D // 2, T), u32),
            pltpu.VMEM((D // 2, T), u32),
            pltpu.VMEM((8, S), f32),
            pltpu.VMEM((8, S), f32),
            pltpu.SemaphoreType.DMA((3,)),
            pltpu.SemaphoreType.DMA((9,)),
            pltpu.SemaphoreType.DMA((NTILE,)),
        ],
        compiler_params=pltpu.CompilerParams(vmem_limit_bytes=64 * 1024 * 1024),
    )(A_x.reshape(S, D).T, A_wqkv, jnp.transpose(A_w_phi, (1, 0, 2)), A_wo, B_w1, B_b1, B_w2.T, B_b2)
    return outT.T.reshape(1, S, D)
```
